```python
import jax
import jax.numpy as jnp

def _softmax(x, axis=-1):
    return jax.nn.softmax(x, axis=axis)
def _gelu(x):
    return jax.nn.gelu(x, approximate=True)
def _silu(x):
    return jax.nn.silu(x)
def _sigmoid(x):
    return jax.nn.sigmoid(x)
def _layernorm(x, axis=-1, eps=1e-5):
    m = jnp.mean(x, axis=axis, keepdims=True)
    v = jnp.var(x, axis=axis, keepdims=True)
    return (x - m) / jnp.sqrt(v + eps)
def _scatter_add(tgt, idx, src, axis=0):
    return tgt.at[idx].add(src)
def _segment_sum(src, seg, n):
    return jax.ops.segment_sum(src, seg, n)
class _Rng:
    def __init__(self, key):
        self._k = key
    def _next(self):
        self._k, sub = jax.random.split(self._k)
        return sub
    def normal(self, shape):
        return jax.random.normal(self._next(), shape, dtype=jnp.bfloat16)
    def randint(self, lo, hi, shape):
        return jax.random.randint(self._next(), shape, lo, hi, dtype=jnp.int32)
    def uniform(self, shape, lo=0.0, hi=1.0):
        return jax.random.uniform(self._next(), shape, jnp.bfloat16, lo, hi)
    def permutation(self, n):
        return jax.random.permutation(self._next(), n)


kernel_name = 'standalone__dcn_v2_cross__recsys'

def setup_inputs():
    _rng = _Rng(jax.random.key(int.from_bytes(__import__("os").urandom(4), "little")))
    _w = (lambda a: (lambda t: t.astype(jnp.bfloat16) if jnp.issubdtype(t.dtype, jnp.floating) else t)(jnp.asarray(a)))
    B, F, D, L = 16384, 26, 128, 6
    Din = min(F * D, 1024)
    return {
        "x0": _w((lambda *s: _rng.normal(s) * 0.05)(B, Din)),
        "ws": _w((lambda *s: _rng.normal(s) * 0.05)(L, Din, Din)),
        "bs": _w((lambda *s: _rng.normal(s) * 0.05)(L, Din)),
    }

def reference(x0, ws, bs):
    x = x0
    for l in range(ws.shape[0]):
        x = x0 * (x @ ws[l] + bs[l]) + x
    return x
```

```python
import jax
import jax.numpy as jnp
import jax.experimental.pallas as pl
import jax.experimental.pallas.tpu as pltpu

BM = 512


def _kernel(x0_ref, ws_ref, bs_ref, o_ref):
    L = ws_ref.shape[0]
    x0 = x0_ref[...].astype(jnp.float32)
    x = x0
    for l in range(L):
        xw = jnp.dot(x.astype(jnp.bfloat16), ws_ref[l], preferred_element_type=jnp.float32)
        b = bs_ref[l:l + 1, :].astype(jnp.float32)
        x = x0 * (xw + b) + x
    o_ref[...] = x.astype(o_ref.dtype)


@jax.jit
def pallas_standalone__dcn_v2_cross__recsys_kernel(x0, ws, bs):
    B, D = x0.shape
    L = ws.shape[0]
    return pl.pallas_call(
        _kernel,
        grid=(B // BM,),
        in_specs=[
            pl.BlockSpec((BM, D), lambda i: (i, 0)),
            pl.BlockSpec((L, D, D), lambda i: (0, 0, 0)),
            pl.BlockSpec((L, D), lambda i: (0, 0)),
        ],
        out_specs=pl.BlockSpec((BM, D), lambda i: (i, 0)),
        out_shape=jax.ShapeDtypeStruct((B, D), x0.dtype),
        compiler_params=pltpu.CompilerParams(
            dimension_semantics=("parallel",),
            vmem_limit_bytes=100 * 1024 * 1024,
        ),
    )(x0, ws, bs)
```

```python
import jax
import jax.numpy as jnp
from jax import lax
import jax.experimental.pallas as pl
import jax.experimental.pallas.tpu as pltpu

SB = 640
NSUB = 1
BM = SB * NSUB
P = 384


def _kernel(x0_hbm, ws_hbm, bs_hbm, o_hbm, w_v, b_v, x_v, o_v, acc, sem, xsem, osem):
    L = ws_hbm.shape[0]
    nblk = (x0_hbm.shape[0] - P) // BM + 1

    def layers(slot, u, hooks=None):
        x0 = x_v[slot, u * SB:(u + 1) * SB, :].astype(jnp.float32)
        x = x0
        for l in range(L):
            if hooks is not None and l in hooks:
                hooks[l]()
            xw = jnp.dot(x.astype(jnp.bfloat16), w_v[l],
                         preferred_element_type=jnp.float32)
            x = x0 * (xw + b_v[l:l + 1, :].astype(jnp.float32)) + x
        return x.astype(o_v.dtype)

    def xcopy(i, slot):
        return pltpu.make_async_copy(
            x0_hbm.at[pl.ds(pl.multiple_of(P + (i - 1) * BM, 64), BM)], x_v.at[slot], xsem.at[slot])

    def ocopy(i, slot, u):
        return pltpu.make_async_copy(
            o_v.at[slot, pl.ds(u * SB, SB)],
            o_hbm.at[pl.ds(pl.multiple_of(P + (i - 1) * BM + u * SB, 64), SB)], osem.at[slot, u])

    def finish(i, slot, u, r):
        o_v[slot, u * SB:(u + 1) * SB, :] = r
        ocopy(i, slot, u).start()

    def wcopy(l):
        return pltpu.make_async_copy(ws_hbm.at[l], w_v.at[l], sem.at[l])

    x_first = pltpu.make_async_copy(x0_hbm.at[pl.ds(0, P)], x_v.at[0, pl.ds(0, P)], xsem.at[0])
    o_first = pltpu.make_async_copy(o_v.at[0, pl.ds(0, P)], o_hbm.at[pl.ds(0, P)], osem.at[0, 0])
    bcopy = pltpu.make_async_copy(bs_hbm, b_v, sem.at[L])
    x_first.start()
    bcopy.start()
    wcopy(0).start()
    x_first.wait()
    bcopy.wait()
    acc[...] = x_v[0, :P, :].astype(jnp.float32)

    def first(l, carry):
        wcopy(l).wait()

        @pl.when(l + 1 < L)
        def _():
            wcopy(l + 1).start()

        @pl.when(l + 1 == L)
        def _():
            xcopy(1, 1).start()

        x = acc[...]
        xw = jnp.dot(x.astype(jnp.bfloat16), w_v[l], preferred_element_type=jnp.float32)
        bf = b_v[...].astype(jnp.float32)
        row = lax.broadcasted_iota(jnp.int32, bf.shape, 0)
        b = jnp.sum(jnp.where(row == l, bf, 0.0), axis=0, keepdims=True)
        acc[...] = x_v[0, :P, :].astype(jnp.float32) * (xw + b) + x
        return carry

    lax.fori_loop(0, L, first, 0)
    o_v[0, :P, :] = acc[...].astype(o_v.dtype)
    o_first.start()

    def body(i, carry):
        slot = i % 2
        xcopy(i, slot).wait()

        @pl.when(i == 2)
        def _():
            o_first.wait()

        @pl.when(i > 2)
        def _():
            for u in range(NSUB):
                ocopy(i - 2, slot, u).wait()

        @pl.when(i + 1 < nblk)
        def _():
            xcopy(i + 1, 1 - slot).start()

        for u in range(NSUB):
            finish(i, slot, u, layers(slot, u))
        return carry

    lax.fori_loop(1, nblk, body, 0)
    for i in (nblk - 2, nblk - 1):
        for u in range(NSUB):
            ocopy(i, i % 2, u).wait()


@jax.jit
def pallas_standalone__dcn_v2_cross__recsys_kernel(x0, ws, bs):
    B, D = x0.shape
    L = ws.shape[0]
    assert (B - P) % BM == 0 and (B - P) // BM >= 2 and P <= SB
    return pl.pallas_call(
        _kernel,
        in_specs=[pl.BlockSpec(memory_space=pl.ANY)] * 3,
        out_specs=pl.BlockSpec(memory_space=pl.ANY),
        out_shape=jax.ShapeDtypeStruct((B, D), x0.dtype),
        scratch_shapes=[
            pltpu.VMEM((L, D, D), ws.dtype),
            pltpu.VMEM((L, D), bs.dtype),
            pltpu.VMEM((2, BM, D), x0.dtype),
            pltpu.VMEM((2, BM, D), x0.dtype),
            pltpu.VMEM((P, D), jnp.float32),
            pltpu.SemaphoreType.DMA((1 + L,)),
            pltpu.SemaphoreType.DMA((2,)),
            pltpu.SemaphoreType.DMA((2, NSUB)),
        ],
        compiler_params=pltpu.CompilerParams(vmem_limit_bytes=100 * 1024 * 1024),
    )(x0, ws, bs)
```
